```python
import jax
import jax.numpy as jnp

def _softmax(x, axis=-1):
    return jax.nn.softmax(x, axis=axis)
def _gelu(x):
    return jax.nn.gelu(x, approximate=True)
def _silu(x):
    return jax.nn.silu(x)
def _sigmoid(x):
    return jax.nn.sigmoid(x)
def _layernorm(x, axis=-1, eps=1e-5):
    m = jnp.mean(x, axis=axis, keepdims=True)
    v = jnp.var(x, axis=axis, keepdims=True)
    return (x - m) / jnp.sqrt(v + eps)
def _scatter_add(tgt, idx, src, axis=0):
    return tgt.at[idx].add(src)
def _segment_sum(src, seg, n):
    return jax.ops.segment_sum(src, seg, n)
class _Rng:
    def __init__(self, key):
        self._k = key
    def _next(self):
        self._k, sub = jax.random.split(self._k)
        return sub
    def normal(self, shape):
        return jax.random.normal(self._next(), shape, dtype=jnp.bfloat16)
    def randint(self, lo, hi, shape):
        return jax.random.randint(self._next(), shape, lo, hi, dtype=jnp.int32)
    def uniform(self, shape, lo=0.0, hi=1.0):
        return jax.random.uniform(self._next(), shape, jnp.bfloat16, lo, hi)
    def permutation(self, n):
        return jax.random.permutation(self._next(), n)


kernel_name = 'interleave_layers__sliding_block_cached__dense_activation_gelu__decode'

def _fwd_setup_inputs():
    _rng = _Rng(jax.random.key(int.from_bytes(__import__("os").urandom(4), "little")))
    _w = (lambda a: (lambda t: t.astype(jnp.bfloat16) if jnp.issubdtype(t.dtype, jnp.floating) else t)(jnp.asarray(a)))
    def _A_setup():
        B, Sq, D = 2, 1, 512
        Hq, Hkv, Sk, Dh = 32, 8, 32768, 128
        assert Hq % Hkv == 0, (Hq, Hkv)
        return {
            "x": _w((lambda *s: _rng.normal(s) * 0.05)(B, Sq, D)),
            "k_cache": _w((lambda *s: _rng.normal(s) * 0.05)(B, Hkv, Sk, Dh)),
            "v_cache": _w((lambda *s: _rng.normal(s) * 0.05)(B, Hkv, Sk, Dh)),
            "wq": _w((lambda *s: _rng.normal(s) * 0.05)(D, Hq * Dh) * (D ** -0.5)),
            "wo": _w((lambda *s: _rng.normal(s) * 0.05)(Hq * Dh, D) * ((Hq * Dh) ** -0.5)),
        }
    _A_in = _A_setup()

    def _B_setup():
        B, S, D, F = 2, 1, 512, 1792
        return {
            "x": _w((lambda *s: _rng.normal(s) * 0.05)(B, S, D)),
            "w1": _w((lambda *s: _rng.normal(s) * 0.05)(D, F) * (D ** -0.5)),
            "b1": _w((lambda *s: _rng.normal(s) * 0.05)(F) * 0.01),
            "w2": _w((lambda *s: _rng.normal(s) * 0.05)(F, D) * (F ** -0.5)),
            "b2": _w((lambda *s: _rng.normal(s) * 0.05)(D) * 0.01),
        }
    _B_in = _B_setup()

    return {
        "A_x": _A_in["x"],
        "A_k_cache": _A_in["k_cache"],
        "A_v_cache": _A_in["v_cache"],
        "A_wq": _A_in["wq"],
        "A_wo": _A_in["wo"],
        "B_x": _B_in["x"],
        "B_w1": _B_in["w1"],
        "B_b1": _B_in["b1"],
        "B_w2": _B_in["w2"],
        "B_b2": _B_in["b2"],
    }

def _fwd_reference(A_x, A_k_cache, A_v_cache, A_wq, A_wo, B_x, B_w1, B_b1, B_w2, B_b2):
    def _A_ref(x, k_cache, v_cache, wq, wo):
        B, Sq, D = x.shape
        Hq, Dh = 32, 128
        Hkv, Sk = k_cache.shape[1], k_cache.shape[2]
        W = min(4096, max(256, Sk // 4))
        rep = Hq // Hkv
        q = (lambda x, *d: x.transpose(*d))((x @ wq).reshape(B, Sq, Hq, Dh), 0, 2, 1, 3)
        k = jnp.repeat(k_cache[:, :, Sk - W:, :], rep, axis=1)
        v = jnp.repeat(v_cache[:, :, Sk - W:, :], rep, axis=1)
        scores = jnp.einsum("bhqd,bhkd->bhqk", q, k) * (Dh ** -0.5)
        p = _softmax(scores, axis=-1)
        o = jnp.einsum("bhqk,bhkd->bhqd", p, v)
        return (lambda x, *d: x.transpose(*d))(o, 0, 2, 1, 3).reshape(B, Sq, Hq * Dh) @ wo

    def _B_ref(x, w1, b1, w2, b2):
        h = jnp.einsum("bsd,df->bsf", x, w1) + b1
        h = _gelu(h)
        return jnp.einsum("bsf,fd->bsd", h, w2) + b2

    x = A_x
    x = x + _A_ref(_layernorm(x, axis=-1), A_k_cache, A_v_cache, A_wq, A_wo)
    x = x + _B_ref(_layernorm(x, axis=-1), B_w1, B_b1, B_w2, B_b2)
    x = x + _A_ref(_layernorm(x, axis=-1), A_k_cache, A_v_cache, A_wq, A_wo)
    x = x + _B_ref(_layernorm(x, axis=-1), B_w1, B_b1, B_w2, B_b2)
    return x


def setup_inputs():
    _inp = _fwd_setup_inputs()
    _gk = jax.random.fold_in(jax.random.key(int.from_bytes(__import__("os").urandom(4), "little")), 2**31 - 1)
    _shapes = [[2, 1, 512]]
    _dtypes = ['bfloat16']
    _gks = jax.random.split(_gk, len(_shapes))
    _gs = [jax.random.normal(k, s, dtype=jnp.dtype(d)) * 0.05 for k, s, d in zip(_gks, _shapes, _dtypes)]
    _inp["grad_out"] = _gs[0]
    return _inp

def reference(A_x, A_k_cache, A_v_cache, A_wq, A_wo, B_w1, B_b1, B_w2, B_b2, B_x, grad_out):
    _const = dict(B_x=B_x)
    def _f(*_d):
        return _fwd_reference(**{'A_x': _d[0], 'A_k_cache': _d[1], 'A_v_cache': _d[2], 'A_wq': _d[3], 'A_wo': _d[4], 'B_w1': _d[5], 'B_b1': _d[6], 'B_w2': _d[7], 'B_b2': _d[8], **_const})
    _out, _vjp = jax.vjp(_f, A_x, A_k_cache, A_v_cache, A_wq, A_wo, B_w1, B_b1, B_w2, B_b2)
    _grads = _vjp(grad_out)
    _out0 = jnp.asarray(_out)
    return (_out0, *[jnp.asarray(_g) for _g in _grads])
```

```python
import math

import jax
import jax.numpy as jnp
import jax.experimental.pallas as pl
import jax.experimental.pallas.tpu as pltpu

_F32 = jnp.float32
_BF16 = jnp.bfloat16

_NN = (((1,), (0,)), ((), ()))
_NT = (((1,), (1,)), ((), ()))
_TN = (((0,), (0,)), ((), ()))

_LN_EPS = 1e-5
_GELU_C = math.sqrt(2.0 / math.pi)
_GELU_A = 0.044715

_ROWS = 8


def _dot(a, b, dims):
    return jax.lax.dot_general(a.astype(_BF16), b.astype(_BF16), dims,
                               preferred_element_type=_F32)


def _ln_fwd(x):
    mu = jnp.mean(x, axis=-1, keepdims=True)
    xc = x - mu
    var = jnp.mean(xc * xc, axis=-1, keepdims=True)
    r = jax.lax.rsqrt(var + _LN_EPS)
    return xc * r, r


def _ln_bwd(dy, y, r):
    m1 = jnp.mean(dy, axis=-1, keepdims=True)
    m2 = jnp.mean(dy * y, axis=-1, keepdims=True)
    return r * (dy - m1 - y * m2)


def _gelu_fwd(h):
    t = jnp.tanh(_GELU_C * (h + _GELU_A * h * h * h))
    return 0.5 * h * (1.0 + t), t


def _gelu_grad(h, t):
    return 0.5 * (1.0 + t) + 0.5 * h * (1.0 - t * t) * _GELU_C * (1.0 + 3.0 * _GELU_A * h * h)


@jax.jit
def pallas_interleave_layers__sliding_block_cached__dense_activation_gelu__decode_kernel(
    A_x: jax.Array,
    A_k_cache: jax.Array,
    A_v_cache: jax.Array,
    A_wq: jax.Array,
    A_wo: jax.Array,
    B_x: jax.Array,
    B_w1: jax.Array,
    B_b1: jax.Array,
    B_w2: jax.Array,
    B_b2: jax.Array,
    grad_out: jax.Array,
):
    del B_x
    B, Sq, D = A_x.shape
    assert Sq == 1 and B <= _ROWS
    _, Hkv, Sk, Dh = A_k_cache.shape
    Hq = 32
    assert Dh == 128 and A_wq.shape == (D, Hq * Dh)
    rep = Hq // Hkv
    assert rep <= _ROWS
    W = min(4096, max(256, Sk // 4))
    F = B_w1.shape[1]
    BH = B * Hkv
    HD = Hq * Dh
    scale = Dh ** -0.5
    Z0 = Sk - W
    ZC = 128
    assert Z0 % ZC == 0 and W % ZC == 0
    n_zc = Z0 // ZC
    n_wc = W // ZC
    Z_INIT = 28
    Z_STEP = 2
    Z_DONE = Z_INIT + 3 * BH * Z_STEP
    assert Z_DONE <= n_zc

    def kernel(x_ref, g_ref, b1_ref, b2_ref,
               k_hbm, v_hbm, wq_hbm, wo_hbm, w1_hbm, w2_hbm,
               out_ref, dx_ref, dk_hbm, dv_hbm, dwq_hbm, dwo_hbm, dw1_hbm,
               db1_ref, dw2_hbm, db2_ref,
               kbuf, vbuf, wq, wo, w1, w2, dwq_s, dwo_s, dw1_s, dw2_s, zbuf,
               p_s, ds_s, q_s, do_s, hd_s, row_s, pad_s,
               wsem, ksem, vsem, zsem, osem):
        w_in = [pltpu.make_async_copy(src, dst, wsem.at[i]) for i, (src, dst) in
                enumerate(((wq_hbm, wq), (wo_hbm, wo), (w1_hbm, w1), (w2_hbm, w2)))]

        def k_in(i):
            return pltpu.make_async_copy(k_hbm.at[i, pl.ds(Z0, W), :], kbuf.at[i], ksem.at[i])

        def v_in(i):
            return pltpu.make_async_copy(v_hbm.at[i, pl.ds(Z0, W), :], vbuf.at[i], vsem.at[i])

        def win_out(c):
            r0 = pl.multiple_of(c * ZC, ZC)
            return [pltpu.make_async_copy(src.at[:, pl.ds(r0, ZC), :],
                                          dst.at[:, pl.ds(Z0 + r0, ZC), :], zsem.at[1])
                    for src, dst in ((kbuf, dk_hbm), (vbuf, dv_hbm))]

        def z_out(c):
            r0 = pl.multiple_of(c * ZC, ZC)
            return [pltpu.make_async_copy(zbuf, dst.at[:, pl.ds(r0, ZC), :], zsem.at[0])
                    for dst in (dk_hbm, dv_hbm)]

        def run_range(make, lo, hi, method):
            def body(c, carry):
                for cp in make(c):
                    getattr(cp, method)()
                return carry
            jax.lax.fori_loop(lo, hi, body, 0)

        def z_step(loop_idx, i):
            c0 = Z_INIT + (loop_idx * BH + i) * Z_STEP
            for j in range(Z_STEP):
                for cp in z_out(c0 + j):
                    cp.start()

        w_out = [pltpu.make_async_copy(src, dst, osem.at[i]) for i, (src, dst) in
                 enumerate(((dwq_s, dwq_hbm), (dwo_s, dwo_hbm), (dw1_s, dw1_hbm), (dw2_s, dw2_hbm)))]

        for cp in w_in:
            cp.start()
        for i in range(BH):
            k_in(i).start()
            v_in(i).start()

        zbuf[...] = jnp.zeros(zbuf.shape, zbuf.dtype)
        q_s[...] = jnp.zeros(q_s.shape, q_s.dtype)
        do_s[...] = jnp.zeros(do_s.shape, do_s.dtype)
        row_s[...] = jnp.zeros(row_s.shape, row_s.dtype)
        pad_s[...] = jnp.zeros(pad_s.shape, pad_s.dtype)
        pad_s[0, 0:B, :] = x_ref[...].astype(_F32)
        pad_s[1, 0:B, :] = g_ref[...].astype(_F32)
        x0 = pad_s[0]
        gout = pad_s[1]
        b1 = b1_ref[...].astype(_F32).reshape(1, F)
        b2 = b2_ref[...].astype(_F32).reshape(1, D)

        def rows_to_heads(row, dst, l):
            for b in range(B):
                for h in range(Hkv):
                    for j in range(rep):
                        c = (h * rep + j) * Dh
                        dst[l, b * Hkv + h, j:j + 1, :] = row[b:b + 1, c:c + Dh]

        def heads_to_rows(slot):
            for b in range(B):
                for h in range(Hkv):
                    for j in range(rep):
                        c = (h * rep + j) * Dh
                        row_s[slot, b:b + 1, c:c + Dh] = hd_s[b * Hkv + h, j:j + 1, :]
            return row_s[slot]

        def attn_fwd(x, l, first):
            n, r = _ln_fwd(x)
            if first:
                w_in[0].wait()
            q = _dot(n, wq[...], _NN)
            rows_to_heads(q, q_s, l)

            def body(i, carry):
                if first:
                    k_in(i).wait()
                    v_in(i).wait()

                    @pl.when(i == BH - 2)
                    def _():
                        run_range(z_out, 0, Z_INIT, "start")
                else:
                    z_step(0, i)
                s = _dot(q_s[l, i], kbuf[i], _NT) * scale
                m = jnp.max(s, axis=-1, keepdims=True)
                e = jnp.exp(s - m)
                p = e / jnp.sum(e, axis=-1, keepdims=True)
                p_s[l, i] = p
                hd_s[i] = _dot(p, vbuf[i], _NN)
                return carry

            jax.lax.fori_loop(0, BH, body, 0)
            o = heads_to_rows(l)
            if first:
                w_in[1].wait()
            a = _dot(o, wo[...], _NN)
            return x + a, n, r, o

        def mlp_fwd(x, first):
            n, r = _ln_fwd(x)
            if first:
                w_in[2].wait()
                w_in[3].wait()
            h = _dot(n, w1[...], _NN) + b1
            g, t = _gelu_fwd(h)
            m = _dot(g, w2[...], _NN) + b2
            return x + m, n, r, h, g, t

        x1, n1, r1, o1 = attn_fwd(x0, 0, True)
        x2, n2, r2, h2, g2, t2 = mlp_fwd(x1, True)
        x3, n3, r3, o3 = attn_fwd(x2, 1, False)
        x4, n4, r4, h4, g4, t4 = mlp_fwd(x3, False)
        out_ref[...] = x4[0:B, :].astype(out_ref.dtype)

        def mlp_bwd(dy, n, r, h, t):
            dg = _dot(dy, w2[...], _NT)
            dh = dg * _gelu_grad(h, t)
            dn = _dot(dh, w1[...], _NT)
            return dy + _ln_bwd(dn, n, r), dh

        def attn_bwd(dy, n, r, l, last):
            do = _dot(dy, wo[...], _NT)
            rows_to_heads(do, do_s, l)

            def body(i, carry):
                z_step(2 if last else 1, i)
                dp = _dot(do_s[l, i], vbuf[i], _NT)
                p = p_s[l, i]
                delta = jnp.sum(p * dp, axis=-1, keepdims=True)
                ds = p * (dp - delta) * scale
                hd_s[i] = _dot(ds, kbuf[i], _NN)
                if not last:
                    ds_s[i] = ds
                else:
                    dsc = jnp.concatenate([ds, ds_s[i]], axis=0)
                    qc = jnp.concatenate([q_s[0, i], q_s[1, i]], axis=0)
                    kbuf[i] = _dot(dsc, qc, _TN).astype(kbuf.dtype)
                    pc = jnp.concatenate([p, p_s[1, i]], axis=0)
                    doc = jnp.concatenate([do_s[0, i], do_s[1, i]], axis=0)
                    vbuf[i] = _dot(pc, doc, _TN).astype(vbuf.dtype)
                return carry

            jax.lax.fori_loop(0, BH, body, 0)
            if last:
                run_range(win_out, 0, n_wc, "start")
            dq = heads_to_rows(2 + l)
            dn = _dot(dq, wq[...], _NT)
            return dy + _ln_bwd(dn, n, r), dq

        def cat(a, b):
            return jnp.concatenate([a, b], axis=0)

        dx3, dh4 = mlp_bwd(gout, n4, r4, h4, t4)
        dx2, dq3 = attn_bwd(dx3, n3, r3, 1, False)
        dx1, dh2 = mlp_bwd(dx2, n2, r2, h2, t2)

        dw2_s[...] = _dot(cat(g2, g4), cat(dx2, gout), _TN).astype(dw2_s.dtype)
        w_out[3].start()
        dw1_s[...] = _dot(cat(n2, n4), cat(dh2, dh4), _TN).astype(dw1_s.dtype)
        w_out[2].start()
        db2_ref[...] = jnp.sum(dx2 + gout, axis=0).astype(db2_ref.dtype)
        db1_ref[...] = jnp.sum(dh2 + dh4, axis=0).astype(db1_ref.dtype)
        dwo_s[...] = _dot(cat(o1, o3), cat(dx1, dx3), _TN).astype(dwo_s.dtype)
        w_out[1].start()

        dx0, dq1 = attn_bwd(dx1, n1, r1, 0, True)
        dx_ref[...] = dx0[0:B, :].astype(dx_ref.dtype)
        dwq_s[...] = _dot(cat(n1, n3), cat(dq1, dq3), _TN).astype(dwq_s.dtype)
        w_out[0].start()
        run_range(z_out, Z_DONE, n_zc, "start")

        for cp in w_out:
            cp.wait()
        run_range(win_out, 0, n_wc, "wait")
        run_range(z_out, 0, n_zc, "wait")

    vmem = pl.BlockSpec(memory_space=pltpu.VMEM)
    hbm = pl.BlockSpec(memory_space=pl.ANY)
    dt = A_x.dtype
    out_shape = (
        jax.ShapeDtypeStruct((B, D), dt),
        jax.ShapeDtypeStruct((B, D), dt),
        jax.ShapeDtypeStruct((BH, Sk, Dh), dt),
        jax.ShapeDtypeStruct((BH, Sk, Dh), dt),
        jax.ShapeDtypeStruct(A_wq.shape, dt),
        jax.ShapeDtypeStruct(A_wo.shape, dt),
        jax.ShapeDtypeStruct(B_w1.shape, dt),
        jax.ShapeDtypeStruct((F,), dt),
        jax.ShapeDtypeStruct(B_w2.shape, dt),
        jax.ShapeDtypeStruct((D,), dt),
    )
    out_specs = (vmem, vmem, hbm, hbm, hbm, hbm, hbm, vmem, hbm, vmem)
    scratch = [
        pltpu.VMEM((BH, W, Dh), dt),
        pltpu.VMEM((BH, W, Dh), dt),
        pltpu.VMEM(A_wq.shape, dt),
        pltpu.VMEM(A_wo.shape, dt),
        pltpu.VMEM(B_w1.shape, dt),
        pltpu.VMEM(B_w2.shape, dt),
        pltpu.VMEM(A_wq.shape, dt),
        pltpu.VMEM(A_wo.shape, dt),
        pltpu.VMEM(B_w1.shape, dt),
        pltpu.VMEM(B_w2.shape, dt),
        pltpu.VMEM((BH, ZC, Dh), dt),
        pltpu.VMEM((2, BH, _ROWS, W), _F32),
        pltpu.VMEM((BH, _ROWS, W), _F32),
        pltpu.VMEM((2, BH, _ROWS, Dh), _F32),
        pltpu.VMEM((2, BH, _ROWS, Dh), _F32),
        pltpu.VMEM((BH, _ROWS, Dh), _F32),
        pltpu.VMEM((4, _ROWS, HD), _F32),
        pltpu.VMEM((2, _ROWS, D), _F32),
        pltpu.SemaphoreType.DMA((4,)),
        pltpu.SemaphoreType.DMA((BH,)),
        pltpu.SemaphoreType.DMA((BH,)),
        pltpu.SemaphoreType.DMA((2,)),
        pltpu.SemaphoreType.DMA((4,)),
    ]
    outs = pl.pallas_call(
        kernel,
        in_specs=[vmem, vmem, vmem, vmem, hbm, hbm, hbm, hbm, hbm, hbm],
        out_specs=out_specs,
        out_shape=out_shape,
        scratch_shapes=scratch,
        compiler_params=pltpu.CompilerParams(vmem_limit_bytes=110 * 1024 * 1024),
    )(A_x.reshape(B, D), grad_out.reshape(B, D), B_b1, B_b2,
      A_k_cache.reshape(BH, Sk, Dh), A_v_cache.reshape(BH, Sk, Dh), A_wq, A_wo, B_w1, B_w2)
    out, dx, dk, dv, dwq, dwo, dw1, db1, dw2, db2 = outs
    return (out.reshape(A_x.shape), dx.reshape(A_x.shape), dk.reshape(A_k_cache.shape),
            dv.reshape(A_v_cache.shape), dwq, dwo, dw1, db1, dw2, db2)
```

```python
import math

import jax
import jax.numpy as jnp
import jax.experimental.pallas as pl
import jax.experimental.pallas.tpu as pltpu

_F32 = jnp.float32
_BF16 = jnp.bfloat16

_NN = (((1,), (0,)), ((), ()))
_NT = (((1,), (1,)), ((), ()))
_TN = (((0,), (0,)), ((), ()))

_LN_EPS = 1e-5
_GELU_C = math.sqrt(2.0 / math.pi)
_GELU_A = 0.044715

_ROWS = 8


def _dot(a, b, dims):
    return jax.lax.dot_general(a.astype(_BF16), b.astype(_BF16), dims,
                               preferred_element_type=_F32)


def _ln_fwd(x):
    mu = jnp.mean(x, axis=-1, keepdims=True)
    xc = x - mu
    var = jnp.mean(xc * xc, axis=-1, keepdims=True)
    r = jax.lax.rsqrt(var + _LN_EPS)
    return xc * r, r


def _ln_bwd(dy, y, r):
    m1 = jnp.mean(dy, axis=-1, keepdims=True)
    m2 = jnp.mean(dy * y, axis=-1, keepdims=True)
    return r * (dy - m1 - y * m2)


def _gelu_fwd(h):
    t = jnp.tanh(_GELU_C * (h + _GELU_A * h * h * h))
    return 0.5 * h * (1.0 + t), t


def _gelu_grad(h, t):
    return 0.5 * (1.0 + t) + 0.5 * h * (1.0 - t * t) * _GELU_C * (1.0 + 3.0 * _GELU_A * h * h)


@jax.jit
def pallas_interleave_layers__sliding_block_cached__dense_activation_gelu__decode_kernel(
    A_x: jax.Array,
    A_k_cache: jax.Array,
    A_v_cache: jax.Array,
    A_wq: jax.Array,
    A_wo: jax.Array,
    B_x: jax.Array,
    B_w1: jax.Array,
    B_b1: jax.Array,
    B_w2: jax.Array,
    B_b2: jax.Array,
    grad_out: jax.Array,
):
    del B_x
    B, Sq, D = A_x.shape
    assert Sq == 1 and B <= _ROWS
    _, Hkv, Sk, Dh = A_k_cache.shape
    Hq = 32
    assert Dh == 128 and A_wq.shape == (D, Hq * Dh)
    rep = Hq // Hkv
    assert rep <= _ROWS
    W = min(4096, max(256, Sk // 4))
    F = B_w1.shape[1]
    BH = B * Hkv
    HD = Hq * Dh
    scale = Dh ** -0.5
    Z0 = Sk - W

    ZC = 128
    OFF = 40
    assert Z0 % ZC == 0 and W % ZC == 0
    n_zc = Z0 // ZC - 1
    n_wc = W // ZC - 1
    Z_INIT = 28
    Z_STEP = 2
    Z_DONE = Z_INIT + 3 * BH * Z_STEP
    dw_rows = (8, 64, 8, 32)
    dw_n = (D // dw_rows[0], HD // dw_rows[1], D // dw_rows[2], F // dw_rows[3])
    assert D % dw_rows[0] == 0 and HD % dw_rows[1] == 0 and F % dw_rows[3] == 0
    assert dw_n[0] == dw_n[1] == dw_n[2] >= dw_n[3]
    assert Z_DONE + dw_n[0] <= n_zc

    def kernel(x_ref, g_ref, b1_ref, b2_ref,
               k_hbm, v_hbm, wq_hbm, wo_hbm, w1_hbm, w2_hbm,
               out_ref, dx_ref, dk_hbm, dv_hbm, dwq_hbm, dwo_hbm, dw1_hbm,
               db1_ref, dw2_hbm, db2_ref,
               kbuf, vbuf, wq, wo, w1, w2, dwq_s, dwo_s, dw1_s, dw2_s, zbuf,
               p_s, ds_s, q_s, do_s, hd_s, row_s, pad_s,
               wsem, ksem, vsem, zsem, osem):
        w_in = [pltpu.make_async_copy(src, dst, wsem.at[i]) for i, (src, dst) in
                enumerate(((wq_hbm, wq), (wo_hbm, wo), (w1_hbm, w1), (w2_hbm, w2)))]

        def k_in(i):
            return pltpu.make_async_copy(k_hbm.at[i, pl.ds(Z0, W), :], kbuf.at[i], ksem.at[i])

        def v_in(i):
            return pltpu.make_async_copy(v_hbm.at[i, pl.ds(Z0, W), :], vbuf.at[i], vsem.at[i])

        def z_out(c):
            r0 = pl.multiple_of(c * ZC + OFF, 8)
            return [pltpu.make_async_copy(zbuf, dst.at[:, pl.ds(r0, ZC), :], zsem.at[0])
                    for dst in (dk_hbm, dv_hbm)]

        def z_edges():
            t0 = OFF + n_zc * ZC
            return [pltpu.make_async_copy(zbuf.at[:, pl.ds(0, n), :],
                                          dst.at[:, pl.ds(r0, n), :], zsem.at[0])
                    for dst in (dk_hbm, dv_hbm) for r0, n in ((0, OFF), (t0, Z0 - t0))]

        def win_out(c):
            r0 = pl.multiple_of(c * ZC + OFF, 8)
            return [pltpu.make_async_copy(src.at[:, pl.ds(r0, ZC), :],
                                          dst.at[:, pl.ds(Z0 + r0, ZC), :], zsem.at[1])
                    for src, dst in ((kbuf, dk_hbm), (vbuf, dv_hbm))]

        def win_edges():
            t0 = OFF + n_wc * ZC
            return [pltpu.make_async_copy(src.at[:, pl.ds(r0, n), :],
                                          dst.at[:, pl.ds(Z0 + r0, n), :], zsem.at[1])
                    for src, dst in ((kbuf, dk_hbm), (vbuf, dv_hbm))
                    for r0, n in ((0, OFF), (t0, W - t0))]

        def dw_out(j, k):
            src, dst = ((dwq_s, dwq_hbm), (dwo_s, dwo_hbm), (dw1_s, dw1_hbm), (dw2_s, dw2_hbm))[j]
            r0 = pl.multiple_of(k * dw_rows[j], dw_rows[j])
            return pltpu.make_async_copy(src.at[pl.ds(r0, dw_rows[j]), :],
                                         dst.at[pl.ds(r0, dw_rows[j]), :], osem.at[j])

        def run_range(make, lo, hi, method):
            def body(c, carry):
                for cp in make(c):
                    getattr(cp, method)()
                return carry
            jax.lax.fori_loop(lo, hi, body, 0)

        def z_step(loop_idx, i):
            c0 = Z_INIT + (loop_idx * BH + i) * Z_STEP
            for j in range(Z_STEP):
                for cp in z_out(c0 + j):
                    cp.start()

        for cp in w_in:
            cp.start()
        for i in range(BH):
            k_in(i).start()
            v_in(i).start()

        zbuf[...] = jnp.zeros(zbuf.shape, zbuf.dtype)
        q_s[...] = jnp.zeros(q_s.shape, q_s.dtype)
        do_s[...] = jnp.zeros(do_s.shape, do_s.dtype)
        row_s[...] = jnp.zeros(row_s.shape, row_s.dtype)
        pad_s[...] = jnp.zeros(pad_s.shape, pad_s.dtype)
        pad_s[0, 0:B, :] = x_ref[...].astype(_F32)
        pad_s[1, 0:B, :] = g_ref[...].astype(_F32)
        x0 = pad_s[0]
        gout = pad_s[1]
        b1 = b1_ref[...].astype(_F32).reshape(1, F)
        b2 = b2_ref[...].astype(_F32).reshape(1, D)

        def rows_to_heads(row, dst, l):
            for b in range(B):
                for h in range(Hkv):
                    for j in range(rep):
                        c = (h * rep + j) * Dh
                        dst[l, b * Hkv + h, j:j + 1, :] = row[b:b + 1, c:c + Dh]

        def heads_to_rows(slot):
            for b in range(B):
                for h in range(Hkv):
                    for j in range(rep):
                        c = (h * rep + j) * Dh
                        row_s[slot, b:b + 1, c:c + Dh] = hd_s[b * Hkv + h, j:j + 1, :]
            return row_s[slot]

        def attn_fwd(x, l, first):
            n, r = _ln_fwd(x)
            if first:
                w_in[0].wait()
            q = _dot(n, wq[...], _NN)
            rows_to_heads(q, q_s, l)

            def body(i, carry):
                if first:
                    k_in(i).wait()
                    v_in(i).wait()

                    @pl.when(i == BH - 2)
                    def _():
                        run_range(z_out, 0, Z_INIT, "start")
                else:
                    z_step(0, i)
                s = _dot(q_s[l, i], kbuf[i], _NT) * scale
                m = jnp.max(s, axis=-1, keepdims=True)
                e = jnp.exp(s - m)
                p = e / jnp.sum(e, axis=-1, keepdims=True)
                p_s[l, i] = p
                hd_s[i] = _dot(p, vbuf[i], _NN)
                return carry

            jax.lax.fori_loop(0, BH, body, 0)
            o = heads_to_rows(l)
            if first:
                w_in[1].wait()
            a = _dot(o, wo[...], _NN)
            return x + a, n, r, o

        def mlp_fwd(x, first):
            n, r = _ln_fwd(x)
            if first:
                w_in[2].wait()
                w_in[3].wait()
            h = _dot(n, w1[...], _NN) + b1
            g, t = _gelu_fwd(h)
            m = _dot(g, w2[...], _NN) + b2
            return x + m, n, r, h, g, t

        x1, n1, r1, o1 = attn_fwd(x0, 0, True)
        x2, n2, r2, h2, g2, t2 = mlp_fwd(x1, True)
        x3, n3, r3, o3 = attn_fwd(x2, 1, False)
        x4, n4, r4, h4, g4, t4 = mlp_fwd(x3, False)
        out_ref[...] = x4[0:B, :].astype(out_ref.dtype)

        def mlp_bwd(dy, n, r, h, t):
            dg = _dot(dy, w2[...], _NT)
            dh = dg * _gelu_grad(h, t)
            dn = _dot(dh, w1[...], _NT)
            return dy + _ln_bwd(dn, n, r), dh

        def attn_bwd(dy, n, r, l, last):
            do = _dot(dy, wo[...], _NT)
            rows_to_heads(do, do_s, l)

            def body(i, carry):
                z_step(2 if last else 1, i)
                dp = _dot(do_s[l, i], vbuf[i], _NT)
                p = p_s[l, i]
                delta = jnp.sum(p * dp, axis=-1, keepdims=True)
                ds = p * (dp - delta) * scale
                hd_s[i] = _dot(ds, kbuf[i], _NN)
                if not last:
                    ds_s[i] = ds
                else:
                    dsc = jnp.concatenate([ds, ds_s[i]], axis=0)
                    qc = jnp.concatenate([q_s[0, i], q_s[1, i]], axis=0)
                    kbuf[i] = _dot(dsc, qc, _TN).astype(kbuf.dtype)
                    pc = jnp.concatenate([p, p_s[1, i]], axis=0)
                    doc = jnp.concatenate([do_s[0, i], do_s[1, i]], axis=0)
                    vbuf[i] = _dot(pc, doc, _TN).astype(vbuf.dtype)
                return carry

            jax.lax.fori_loop(0, BH, body, 0)
            if last:
                run_range(win_out, 0, n_wc, "start")
                for cp in win_edges():
                    cp.start()
            dq = heads_to_rows(2 + l)
            dn = _dot(dq, wq[...], _NT)
            return dy + _ln_bwd(dn, n, r), dq

        def cat(a, b):
            return jnp.concatenate([a, b], axis=0)

        dx3, dh4 = mlp_bwd(gout, n4, r4, h4, t4)
        dx2, dq3 = attn_bwd(dx3, n3, r3, 1, False)
        dx1, dh2 = mlp_bwd(dx2, n2, r2, h2, t2)

        dw2_s[...] = _dot(cat(g2, g4), cat(dx2, gout), _TN).astype(dw2_s.dtype)
        dw1_s[...] = _dot(cat(n2, n4), cat(dh2, dh4), _TN).astype(dw1_s.dtype)
        db2_ref[...] = jnp.sum(dx2 + gout, axis=0).astype(db2_ref.dtype)
        db1_ref[...] = jnp.sum(dh2 + dh4, axis=0).astype(db1_ref.dtype)
        dwo_s[...] = _dot(cat(o1, o3), cat(dx1, dx3), _TN).astype(dwo_s.dtype)

        dx0, dq1 = attn_bwd(dx1, n1, r1, 0, True)
        dx_ref[...] = dx0[0:B, :].astype(dx_ref.dtype)
        dwq_s[...] = _dot(cat(n1, n3), cat(dq1, dq3), _TN).astype(dwq_s.dtype)

        run_range(lambda k: z_out(Z_DONE + k) + [dw_out(j, k) for j in range(4)],
                  0, dw_n[3], "start")
        run_range(lambda k: z_out(Z_DONE + k) + [dw_out(j, k) for j in range(3)],
                  dw_n[3], dw_n[0], "start")
        run_range(z_out, Z_DONE + dw_n[0], n_zc, "start")
        for cp in z_edges():
            cp.start()

        for j in range(4):
            run_range(lambda k, j=j: [dw_out(j, k)], 0, dw_n[j], "wait")
        run_range(win_out, 0, n_wc, "wait")
        for cp in win_edges():
            cp.wait()
        run_range(z_out, 0, n_zc, "wait")
        for cp in z_edges():
            cp.wait()

    vmem = pl.BlockSpec(memory_space=pltpu.VMEM)
    hbm = pl.BlockSpec(memory_space=pl.ANY)
    dt = A_x.dtype
    out_shape = (
        jax.ShapeDtypeStruct((B, D), dt),
        jax.ShapeDtypeStruct((B, D), dt),
        jax.ShapeDtypeStruct((BH, Sk, Dh), dt),
        jax.ShapeDtypeStruct((BH, Sk, Dh), dt),
        jax.ShapeDtypeStruct(A_wq.shape, dt),
        jax.ShapeDtypeStruct(A_wo.shape, dt),
        jax.ShapeDtypeStruct(B_w1.shape, dt),
        jax.ShapeDtypeStruct((F,), dt),
        jax.ShapeDtypeStruct(B_w2.shape, dt),
        jax.ShapeDtypeStruct((D,), dt),
    )
    out_specs = (vmem, vmem, hbm, hbm, hbm, hbm, hbm, vmem, hbm, vmem)
    scratch = [
        pltpu.VMEM((BH, W, Dh), dt),
        pltpu.VMEM((BH, W, Dh), dt),
        pltpu.VMEM(A_wq.shape, dt),
        pltpu.VMEM(A_wo.shape, dt),
        pltpu.VMEM(B_w1.shape, dt),
        pltpu.VMEM(B_w2.shape, dt),
        pltpu.VMEM(A_wq.shape, dt),
        pltpu.VMEM(A_wo.shape, dt),
        pltpu.VMEM(B_w1.shape, dt),
        pltpu.VMEM(B_w2.shape, dt),
        pltpu.VMEM((BH, ZC, Dh), dt),
        pltpu.VMEM((2, BH, _ROWS, W), _F32),
        pltpu.VMEM((BH, _ROWS, W), _F32),
        pltpu.VMEM((2, BH, _ROWS, Dh), _F32),
        pltpu.VMEM((2, BH, _ROWS, Dh), _F32),
        pltpu.VMEM((BH, _ROWS, Dh), _F32),
        pltpu.VMEM((4, _ROWS, HD), _F32),
        pltpu.VMEM((2, _ROWS, D), _F32),
        pltpu.SemaphoreType.DMA((4,)),
        pltpu.SemaphoreType.DMA((BH,)),
        pltpu.SemaphoreType.DMA((BH,)),
        pltpu.SemaphoreType.DMA((2,)),
        pltpu.SemaphoreType.DMA((4,)),
    ]
    outs = pl.pallas_call(
        kernel,
        in_specs=[vmem, vmem, vmem, vmem, hbm, hbm, hbm, hbm, hbm, hbm],
        out_specs=out_specs,
        out_shape=out_shape,
        scratch_shapes=scratch,
        compiler_params=pltpu.CompilerParams(vmem_limit_bytes=110 * 1024 * 1024),
    )(A_x.reshape(B, D), grad_out.reshape(B, D), B_b1, B_b2,
      A_k_cache.reshape(BH, Sk, Dh), A_v_cache.reshape(BH, Sk, Dh), A_wq, A_wo, B_w1, B_w2)
    out, dx, dk, dv, dwq, dwo, dw1, db1, dw2, db2 = outs
    return (out.reshape(A_x.shape), dx.reshape(A_x.shape), dk.reshape(A_k_cache.shape),
            dv.reshape(A_v_cache.shape), dwq, dwo, dw1, db1, dw2, db2)
```
